```python
import jax
import jax.numpy as jnp

def _softmax(x, axis=-1):
    return jax.nn.softmax(x, axis=axis)
def _gelu(x):
    return jax.nn.gelu(x, approximate=True)
def _silu(x):
    return jax.nn.silu(x)
def _sigmoid(x):
    return jax.nn.sigmoid(x)
def _layernorm(x, axis=-1, eps=1e-5):
    m = jnp.mean(x, axis=axis, keepdims=True)
    v = jnp.var(x, axis=axis, keepdims=True)
    return (x - m) / jnp.sqrt(v + eps)
def _scatter_add(tgt, idx, src, axis=0):
    return tgt.at[idx].add(src)
def _segment_sum(src, seg, n):
    return jax.ops.segment_sum(src, seg, n)
class _Rng:
    def __init__(self, key):
        self._k = key
    def _next(self):
        self._k, sub = jax.random.split(self._k)
        return sub
    def normal(self, shape):
        return jax.random.normal(self._next(), shape, dtype=jnp.bfloat16)
    def randint(self, lo, hi, shape):
        return jax.random.randint(self._next(), shape, lo, hi, dtype=jnp.int32)
    def uniform(self, shape, lo=0.0, hi=1.0):
        return jax.random.uniform(self._next(), shape, jnp.bfloat16, lo, hi)
    def permutation(self, n):
        return jax.random.permutation(self._next(), n)


kernel_name = 'concat_heads__sliding_block_cached__compressed_kv_cla__decode'

def _fwd_setup_inputs():
    _rng = _Rng(jax.random.key(int.from_bytes(__import__("os").urandom(4), "little")))
    _w = (lambda a: (lambda t: t.astype(jnp.bfloat16) if jnp.issubdtype(t.dtype, jnp.floating) else t)(jnp.asarray(a)))
    def _A_setup():
        B, Sq, D = 1, 1, 640
        Hq, Hkv, Sk, Dh = 32, 32, 4096, 128
        assert Hq % Hkv == 0, (Hq, Hkv)
        return {
            "x": _w((lambda *s: _rng.normal(s) * 0.05)(B, Sq, D)),
            "k_cache": _w((lambda *s: _rng.normal(s) * 0.05)(B, Hkv, Sk, Dh)),
            "v_cache": _w((lambda *s: _rng.normal(s) * 0.05)(B, Hkv, Sk, Dh)),
            "wq": _w((lambda *s: _rng.normal(s) * 0.05)(D, Hq * Dh) * (D ** -0.5)),
            "wo": _w((lambda *s: _rng.normal(s) * 0.05)(Hq * Dh, D) * ((Hq * Dh) ** -0.5)),
        }
    _A_in = _A_setup()

    def _B_setup():
        B, H, Sq, Sk, D, M = 1, 32, 1, 4096, 128, 640
        Dc = 4 * D
        return {
            "x": _w((lambda *s: _rng.normal(s) * 0.05)(B, Sq, M)),
            "c_kv": _w((lambda *s: _rng.normal(s) * 0.05)(B, Sk, Dc)),
            "w_q": _w((lambda *s: _rng.normal(s) * 0.05)(M, H, D) * (M ** -0.5)),
            "w_uk": _w((lambda *s: _rng.normal(s) * 0.05)(Dc, H, D) * (Dc ** -0.5)),
            "w_uv": _w((lambda *s: _rng.normal(s) * 0.05)(Dc, H, D) * (Dc ** -0.5)),
            "w_o": _w((lambda *s: _rng.normal(s) * 0.05)(H, D, M) * ((H * D) ** -0.5)),
        }
    _B_in = _B_setup()

    return {
        "A_x": _A_in["x"],
        "A_k_cache": _A_in["k_cache"],
        "A_v_cache": _A_in["v_cache"],
        "A_wq": _A_in["wq"],
        "A_wo": _A_in["wo"],
        "B_x": _B_in["x"],
        "B_c_kv": _B_in["c_kv"],
        "B_w_q": _B_in["w_q"],
        "B_w_uk": _B_in["w_uk"],
        "B_w_uv": _B_in["w_uv"],
        "B_w_o": _B_in["w_o"],
    }

def _fwd_reference(A_x, A_k_cache, A_v_cache, A_wq, A_wo, B_x, B_c_kv, B_w_q, B_w_uk, B_w_uv, B_w_o):
    def _A_ref(x, k_cache, v_cache, wq, wo):
        B, Sq, D = x.shape
        Hq, Dh = 32, 128
        Hkv, Sk = k_cache.shape[1], k_cache.shape[2]
        W = min(4096, max(256, Sk // 4))
        rep = Hq // Hkv
        q = (lambda x, *d: x.transpose(*d))((x @ wq).reshape(B, Sq, Hq, Dh), 0, 2, 1, 3)
        k = jnp.repeat(k_cache[:, :, Sk - W:, :], rep, axis=1)
        v = jnp.repeat(v_cache[:, :, Sk - W:, :], rep, axis=1)
        scores = jnp.einsum("bhqd,bhkd->bhqk", q, k) * (Dh ** -0.5)
        p = _softmax(scores, axis=-1)
        o = jnp.einsum("bhqk,bhkd->bhqd", p, v)
        return (lambda x, *d: x.transpose(*d))(o, 0, 2, 1, 3).reshape(B, Sq, Hq * Dh) @ wo

    def _B_ref(x, c_kv, w_q, w_uk, w_uv, w_o):
        B, Sq, M = x.shape[0], x.shape[1], x.shape[2]
        Sk = c_kv.shape[1]
        H, D = w_q.shape[1], w_q.shape[2]
        q = jnp.einsum("bqm,mhd->bhqd", x, w_q)
        k = jnp.einsum("bkc,chd->bhkd", c_kv, w_uk)
        v = jnp.einsum("bkc,chd->bhkd", c_kv, w_uv)
        scores = jnp.einsum("bhqd,bhkd->bhqk", q, k) * (D ** -0.5)
        off = Sk - Sq
        qi = jnp.arange(Sq)[:, None]
        kj = jnp.arange(Sk)[None, :]
        cmask = kj <= (qi + off)
        scores = jnp.where(cmask[None, None], scores, -1e9)
        p = _softmax(scores, axis=-1)
        ctx = jnp.einsum("bhqk,bhkd->bhqd", p, v)
        return jnp.einsum("bhqd,hdm->bqm", ctx, w_o)

    a = _A_ref(A_x, A_k_cache, A_v_cache, A_wq, A_wo)
    b = _B_ref(B_x, B_c_kv, B_w_q, B_w_uk, B_w_uv, B_w_o)
    return jnp.concatenate([a, b], axis=-1)


def setup_inputs():
    _inp = _fwd_setup_inputs()
    _gk = jax.random.fold_in(jax.random.key(int.from_bytes(__import__("os").urandom(4), "little")), 2**31 - 1)
    _shapes = [[1, 1, 1280]]
    _dtypes = ['bfloat16']
    _gks = jax.random.split(_gk, len(_shapes))
    _gs = [jax.random.normal(k, s, dtype=jnp.dtype(d)) * 0.05 for k, s, d in zip(_gks, _shapes, _dtypes)]
    _inp["grad_out"] = _gs[0]
    return _inp

def reference(A_x, A_k_cache, A_v_cache, A_wq, A_wo, B_x, B_c_kv, B_w_q, B_w_uk, B_w_uv, B_w_o, grad_out):
    _const = dict()
    def _f(*_d):
        return _fwd_reference(**{'A_x': _d[0], 'A_k_cache': _d[1], 'A_v_cache': _d[2], 'A_wq': _d[3], 'A_wo': _d[4], 'B_x': _d[5], 'B_c_kv': _d[6], 'B_w_q': _d[7], 'B_w_uk': _d[8], 'B_w_uv': _d[9], 'B_w_o': _d[10], **_const})
    _out, _vjp = jax.vjp(_f, A_x, A_k_cache, A_v_cache, A_wq, A_wo, B_x, B_c_kv, B_w_q, B_w_uk, B_w_uv, B_w_o)
    _grads = _vjp(grad_out)
    _out0 = jnp.asarray(_out)
    return (_out0, *[jnp.asarray(_g) for _g in _grads])
```

```python
import jax
import jax.numpy as jnp
import jax.experimental.pallas as pl
import jax.experimental.pallas.tpu as pltpu

bf16 = jnp.bfloat16
f32 = jnp.float32

H = 32
D = 128
M = 640
HD = H * D
SK = 4096
W = 1024
W0 = SK - W
C = 512
SCALE = D ** -0.5

MB = 16
ZH, ZR = 8, 128
NS = 8

NT = (((1,), (1,)), ((), ()))
TN = (((0,), (0,)), ((), ()))


def _dot(a, b):
    return jnp.dot(a, b, preferred_element_type=f32)


def _dot_nt(a, b):
    return jax.lax.dot_general(a, b, NT, preferred_element_type=f32)


def _dot_tn(a, b):
    return jax.lax.dot_general(a, b, TN, preferred_element_type=f32)


def _iota(shape, dim):
    return jax.lax.broadcasted_iota(jnp.int32, shape, dim)


def _softmax_rows(s):
    e = jnp.exp(s - jnp.max(s, axis=1, keepdims=True))
    return e * (1.0 / jnp.sum(e, axis=1, keepdims=True))


def _softmax_bwd_rows(p, dp):
    return p * (dp - jnp.sum(p * dp, axis=1, keepdims=True)) * SCALE


def _put_rows(dst, start, size, val):
    nper = dst.shape[1] // size
    blk = start // size
    dst[blk // nper, pl.ds(pl.multiple_of((blk % nper) * size, size), size)] = val


DEFAULT_CFG = dict(z1=70, z2=130, vback=2)


def _make_kernel(cfg):
    def kernel(
        xa_h, kc_h, vc_h, wq_h, wo_h, xb_h, ckv_h, wbq_h, wuk_h, wuv_h, wbo_h, g_h,
        out_h, dxa_h, dk_h, dv_h, dwq_h, dwo_h, dxb_h, dckv_h, dwbq_h, dwuk_h, dwuv_h, dwbo_h,
        xa_v, xb_v, g_v, k_v, v_v, wq_v, wo_v, ckv_v, wbq_v, wu_v, wbo_v,
        out_v, dxa_v, dxb_v, dk_v, dv_v, dwq_v, dwo_v, dckv_v, dwbq_v, dwu_v, dwbo_v, z_v,
        colb_v, e_v, qd_v, rq_v, qb_v, pd_v, pcd_v, acc_v, t_v, row_v, s_v, dp_v,
        qa_v, doa_v, oa_v, dqa_v, outa_v,
        sem,
    ):
        def cp(src, dst, i):
            return pltpu.make_async_copy(src, dst, sem.at[i])

        def row_chunks(src, dst, size, i):
            return [cp(src.at[pl.ds(j, size)], dst.at[pl.ds(j, size)], i)
                    for j in range(0, dst.shape[0], size)]

        def window(src, dst, h0, h1, i):
            return [cp(src.at[0, h, pl.ds(W0, W), :], dst.at[h], i) for h in range(h0, h1)]

        def start(copies):
            for c in copies:
                c.start()

        def wait(copies):
            for c in copies:
                c.wait()

        vb = H - cfg["vback"]
        r_wbq = row_chunks(wbq_h, wbq_v, 128, 0)
        r_wbq = r_wbq[:1] + [cp(xa_h, xa_v, 0), cp(xb_h, xb_v, 0), cp(g_h, g_v, 0)] + r_wbq[1:]
        r_wuk = row_chunks(wuk_h, wu_v.at[0], 128, 1)
        r_wbo = row_chunks(wbo_h, wbo_v, 8, 2)
        r_wuv = row_chunks(wuv_h, wu_v.at[1], 128, 3)
        r_ckv = row_chunks(ckv_h.at[0], ckv_v, 1024, 0)
        r_wq = row_chunks(wq_h, wq_v, 128, 1)
        r_wo = row_chunks(wo_h, wo_v, 1024, 2)
        r_k = window(kc_h, k_v, 0, H, 3)
        r_v1 = window(vc_h, v_v, 0, vb, 0)
        r_v2 = window(vc_h, v_v, vb, H, 1)

        WS = 2
        w_zero = [cp(z_v, dst.at[0, pl.ds(h, ZH), pl.ds(r, ZR), :], WS)
                  for dst in (dk_h, dv_h) for h in range(0, H, ZH) for r in range(0, W0, ZR)]
        w_dkv = [cp(src.at[pl.ds(h, ZH), pl.ds(r, ZR), :],
                    dst.at[0, pl.ds(h, ZH), pl.ds(W0 + r, ZR), :], WS)
                 for src, dst in ((dk_v, dk_h), (dv_v, dv_h))
                 for h in range(0, H, ZH) for r in range(0, W, ZR)]

        def stream_chunks(src, dst, size):
            return [cp(src.at[:, pl.ds(j, size)], dst.at[:, pl.ds(j, size)], WS)
                    for j in range(0, dst.shape[1], size)]

        w_rest = [cp(dxa_v, dxa_h, WS), cp(dxb_v, dxb_h, WS), cp(out_v, out_h, WS)]
        w_rest += [cp(dwq_v.at[:, pl.ds(r, 8), pl.ds(c, 1024)], dwq_h.at[:, pl.ds(r, 8), pl.ds(c, 1024)], WS)
                   for r in range(0, dwq_h.shape[1], 8) for c in range(0, HD, 1024)]
        w_rest += stream_chunks(dwo_v, dwo_h, 16)
        w_rest += stream_chunks(dwu_v.at[0], dwuk_h, 2)
        w_rest += stream_chunks(dwu_v.at[1], dwuv_h, 2)
        w_rest += stream_chunks(dwbq_v, dwbq_h, 2)
        w_rest += stream_chunks(dwbo_v, dwbo_h, 16)
        w_rest += stream_chunks(dckv_v, dckv_h, 16)

        start(r_wbq)
        start(r_wuk)
        start(r_wbo)
        start(r_wuv)

        z_v[...] = jnp.zeros(z_v.shape, bf16)
        e_v[...] = jnp.where(_iota((HD, 128), 1) == _iota((HD, 128), 0) // H, 1.0, 0.0).astype(bf16)

        wait(r_wbq)
        start(r_ckv)
        colb_v[0] = jnp.broadcast_to(xa_v[0].astype(f32), (128, M)).T
        colb_v[1] = jnp.broadcast_to(xb_v[0].astype(f32), (128, M)).T

        def qb_body(i, acc):
            r = pl.ds(pl.multiple_of(i * MB, MB), MB)
            return acc + jnp.sum(wbq_v[r].astype(f32) * colb_v[1, r, :][:, None, :], axis=0)

        qb_v[0] = jax.lax.fori_loop(0, M // MB, qb_body, jnp.zeros((H, D), f32))

        def absorb(a):
            vec = qb_v[a].astype(bf16)
            own_head = _iota((H, HD), 1) % H == _iota((H, HD), 0)

            def body(j, carry):
                w2 = wu_v[a, pl.ds(j * 128, 128)].reshape(HD, D)
                r = jnp.where(own_head, _dot_nt(vec, w2), 0.0).astype(bf16)
                qd_v[pl.ds(a * H, H), pl.ds(pl.multiple_of(j * 128, 128), 128)] = _dot(r, e_v[...])
                return carry

            jax.lax.fori_loop(0, C // 128, body, 0)

        wait(r_wuk)
        start(r_wq)
        absorb(0)

        wait(r_wbo)
        start(r_wo)
        qb_v[1] = _dot_nt(g_v[0][:, M:], wbo_v[...].reshape(HD, M)).reshape(H, D)

        wait(r_wuv)
        start(r_k)
        absorb(1)

        wait(r_ckv)
        start(r_v1)
        qd = qd_v[...].astype(bf16)
        rq_v[...] = jnp.concatenate([qd[H:], qd[:H]], axis=0)
        sd = _dot_nt(qd, ckv_v[...])
        p_b = _softmax_rows(sd[:H] * SCALE)
        ds_b = _softmax_bwd_rows(p_b, sd[H:])
        pd_v[...] = jnp.concatenate([p_b, ds_b], axis=0).astype(bf16)
        pcd_v[...] = _dot(pd_v[...], ckv_v[...])

        def lform_body(it, carry):
            a = it // 4
            j = it % 4
            blk = pcd_v[pl.ds(pl.multiple_of((1 - a) * H, H), H),
                        pl.ds(pl.multiple_of(j * 128, 128), 128)]
            vec = qb_v[a]
            acc = acc_v[a]
            per = C // NS
            for cc in range(128):
                col = jnp.broadcast_to(blk[:, cc:cc + 1], (H, D))
                dwu_v[a, j * (128 // per) + cc // per, cc % per] = (col * vec).astype(bf16)
                acc = acc + col * wu_v[a, j * 128 + cc].astype(f32)
            acc_v[a] = acc
            return carry

        acc_v[...] = jnp.zeros(acc_v.shape, f32)
        jax.lax.fori_loop(0, 8, lform_body, 0)

        wait(r_wq)
        start(r_v2)
        qa_v[...] = _dot(xa_v[0], wq_v[...]).reshape(H, D)

        dqb = acc_v[0]

        def dwbq_body(i, carry):
            r = pl.ds(pl.multiple_of(i * MB, MB), MB)
            _put_rows(dwbq_v, i * MB, MB, (colb_v[1, r, :][:, None, :] * dqb[None]).astype(bf16))
            t_v[r, :] = jnp.sum(wbq_v[r].astype(f32) * dqb[None], axis=1)
            return carry

        jax.lax.fori_loop(0, M // MB, dwbq_body, 0)
        dxb_v[0] = jax.lax.dot_general(
            jnp.ones((8, D), f32), t_v[...], NT, preferred_element_type=f32,
            precision=jax.lax.Precision.HIGHEST)[0:1].astype(bf16)

        wait(r_wo)
        doa_v[...] = _dot_nt(g_v[0][:, :M], wo_v[...]).reshape(H, D)

        def dckv_body(i, carry):
            blk = pd_v[:, pl.ds(pl.multiple_of(i * 512, 512), 512)]
            _put_rows(dckv_v, i * 512, 512, _dot_tn(blk, rq_v[...]).astype(bf16))
            return carry

        jax.lax.fori_loop(0, SK // 512, dckv_body, 0)

        wait(r_k)

        def s_body(h, carry):
            s_v[pl.ds(h, 1), :] = _dot_nt(qa_v[pl.ds(h, 1), :].astype(bf16), k_v[h])
            return carry

        jax.lax.fori_loop(0, H, s_body, 0, unroll=2)
        s_v[...] = _softmax_rows(s_v[...] * SCALE)

        wait(r_v1)
        start(w_zero[:cfg["z1"]])
        wait(r_v2)

        def dpo_body(h, carry):
            vh = v_v[h]
            dp_v[pl.ds(h, 1), :] = _dot_nt(doa_v[pl.ds(h, 1), :].astype(bf16), vh)
            oa_v[pl.ds(h, 1), :] = _dot(s_v[pl.ds(h, 1), :].astype(bf16), vh)
            return carry

        jax.lax.fori_loop(0, H, dpo_body, 0, unroll=2)
        dp_v[...] = _softmax_bwd_rows(s_v[...], dp_v[...])

        def dq_body(h, carry):
            dqa_v[pl.ds(h, 1), :] = _dot(dp_v[pl.ds(h, 1), :].astype(bf16), k_v[h])
            return carry

        jax.lax.fori_loop(0, H, dq_body, 0, unroll=2)

        p_t = s_v[...].T
        ds_t = dp_v[...].T.astype(bf16)
        head = _iota((H, D), 0)
        qa = qa_v[...]
        for h in range(H):
            dv_v[h] = (p_t[:, h:h + 1] * doa_v[h:h + 1, :]).astype(bf16)
            dk_v[h] = _dot(ds_t, jnp.where(head == h, qa, 0.0).astype(bf16)).astype(bf16)

        start(w_zero[cfg["z1"]:cfg["z2"]])

        dqa_row = dqa_v[...].reshape(1, HD)
        row_v[...] = dqa_row
        outa_v[...] = _dot(oa_v[...].reshape(1, HD).astype(bf16), wo_v[...])
        dxa_v[0] = _dot_nt(dqa_row.astype(bf16), wq_v[...]).astype(bf16)
        out_b = _dot(acc_v[1].reshape(1, HD).astype(bf16), wbo_v[...].reshape(HD, M))
        out_v[0] = jnp.concatenate([outa_v[...], out_b], axis=1).astype(bf16)

        def dwq_body(i, carry):
            xcol = colb_v[0, pl.ds(pl.multiple_of(i * 16, 16), 16), :]
            _put_rows(dwq_v, i * 16, 16, (jnp.concatenate([xcol] * H, axis=1) * row_v[...]).astype(bf16))
            return carry

        jax.lax.fori_loop(0, M // 16, dwq_body, 0)

        def outer(col_ref, grow, dst):
            growf = grow.astype(f32)

            def body(h, carry):
                cb = jnp.broadcast_to(col_ref[pl.ds(h, 1), :], (D, D)).T
                _put_rows(dst, h * D, D, (jnp.concatenate([cb] * (M // 128), axis=1) * growf).astype(bf16))
                return carry

            jax.lax.fori_loop(0, H, body, 0)

        outer(oa_v, g_v[0][:, :M], dwo_v)
        outer(acc_v.at[1], g_v[0][:, M:], dwbo_v)

        start(w_zero[cfg["z2"]:])
        start(w_dkv)
        start(w_rest)
        wait(w_zero)
        wait(w_dkv)
        wait(w_rest)

    return kernel


def make_fn(cfg=None):
    c = dict(DEFAULT_CFG)
    c.update(cfg or {})
    kernel = _make_kernel(c)

    def fn(A_x, A_k_cache, A_v_cache, A_wq, A_wo, B_x, B_c_kv, B_w_q, B_w_uk, B_w_uv, B_w_o, grad_out):
        sds = jax.ShapeDtypeStruct
        sh_dwq = (NS, M // NS, HD)
        sh_dwo = (NS, HD // NS, M)
        sh_dckv = (NS, SK // NS, C)
        sh_dwbq = (NS, M // NS, H, D)
        sh_dwu = (NS, C // NS, H, D)
        out_shape = (
            sds((1, 1, 2 * M), bf16), sds((1, 1, M), bf16),
            sds((1, H, SK, D), bf16), sds((1, H, SK, D), bf16),
            sds(sh_dwq, bf16), sds(sh_dwo, bf16),
            sds((1, 1, M), bf16), sds(sh_dckv, bf16),
            sds(sh_dwbq, bf16), sds(sh_dwu, bf16), sds(sh_dwu, bf16), sds(sh_dwo, bf16),
        )
        vm = pltpu.VMEM
        scratch = [
            vm((1, 1, M), bf16), vm((1, 1, M), bf16), vm((1, 1, 2 * M), bf16),
            vm((H, W, D), bf16), vm((H, W, D), bf16),
            vm((M, HD), bf16), vm((HD, M), bf16), vm((SK, C), bf16),
            vm((M, H, D), bf16), vm((2, C, H, D), bf16), vm((H, D, M), bf16),
            vm((1, 1, 2 * M), bf16), vm((1, 1, M), bf16), vm((1, 1, M), bf16),
            vm((H, W, D), bf16), vm((H, W, D), bf16),
            vm(sh_dwq, bf16), vm(sh_dwo, bf16), vm(sh_dckv, bf16),
            vm(sh_dwbq, bf16), vm((2,) + sh_dwu, bf16), vm(sh_dwo, bf16),
            vm((ZH, ZR, D), bf16),
            vm((2, M, 128), f32),
            vm((HD, 128), bf16),
            vm((2 * H, C), f32),
            vm((2 * H, C), bf16),
            vm((2, H, D), f32),
            vm((2 * H, SK), bf16),
            vm((2 * H, C), f32),
            vm((2, H, D), f32),
            vm((M, D), f32),
            vm((1, HD), f32),
            vm((H, W), f32),
            vm((H, W), f32),
            vm((H, D), f32), vm((H, D), f32), vm((H, D), f32), vm((H, D), f32),
            vm((1, M), f32),
            pltpu.SemaphoreType.DMA((4,)),
        ]
        any_spec = pl.BlockSpec(memory_space=pl.ANY)
        outs = pl.pallas_call(
            kernel,
            out_shape=out_shape,
            in_specs=[any_spec] * 12,
            out_specs=[any_spec] * 12,
            scratch_shapes=scratch,
            compiler_params=pltpu.CompilerParams(vmem_limit_bytes=120 * 1024 * 1024),
        )(A_x, A_k_cache, A_v_cache, A_wq, A_wo, B_x, B_c_kv, B_w_q, B_w_uk, B_w_uv, B_w_o, grad_out)
        out, dxa, dk, dv, dwq, dwo, dxb, dckv, dwbq, dwuk, dwuv, dwbo = outs
        return (out, dxa, dk, dv, dwq.reshape(M, HD), dwo.reshape(HD, M), dxb,
                dckv.reshape(1, SK, C), dwbq.reshape(M, H, D), dwuk.reshape(C, H, D),
                dwuv.reshape(C, H, D), dwbo.reshape(H, D, M))

    return fn


_FN = make_fn()


@jax.jit
def pallas_concat_heads__sliding_block_cached__compressed_kv_cla__decode_kernel(
    A_x, A_k_cache, A_v_cache, A_wq, A_wo, B_x, B_c_kv, B_w_q, B_w_uk, B_w_uv, B_w_o, grad_out,
):
    return _FN(A_x, A_k_cache, A_v_cache, A_wq, A_wo, B_x, B_c_kv, B_w_q, B_w_uk, B_w_uv, B_w_o, grad_out)
```

```python
import jax
import jax.numpy as jnp
import jax.experimental.pallas as pl
import jax.experimental.pallas.tpu as pltpu

bf16 = jnp.bfloat16
f32 = jnp.float32

H = 32
D = 128
M = 640
HD = H * D
SK = 4096
W = 1024
W0 = SK - W
C = 512
SCALE = D ** -0.5

MB = 16
HG = 8
KC = HG * D
RB = 128
NS = 8
ZR = 64
V_LATE = 2
NZ_ROWS = W0 // ZR
NZ = (H // NS) * NZ_ROWS
Z_TOPUP = (72, 108, 130, 165, 200, 240, 280)
W_SEM = 2

NT = (((1,), (1,)), ((), ()))
TN = (((0,), (0,)), ((), ()))


def _dot(a, b):
    return jnp.dot(a, b, preferred_element_type=f32)


def _dot_nt(a, b):
    return jax.lax.dot_general(a, b, NT, preferred_element_type=f32)


def _dot_tn(a, b):
    return jax.lax.dot_general(a, b, TN, preferred_element_type=f32)


def _iota(shape, dim):
    return jax.lax.broadcasted_iota(jnp.int32, shape, dim)


def _softmax_rows(s):
    e = jnp.exp(s - jnp.max(s, axis=1, keepdims=True))
    return e * (1.0 / jnp.sum(e, axis=1, keepdims=True))


def _softmax_bwd_rows(p, dp):
    return p * (dp - jnp.sum(p * dp, axis=1, keepdims=True)) * SCALE


def _blk(i, size):
    return pl.ds(pl.multiple_of(i * size, size), size)


def _put_rows(dst, blk, size, val):
    nper = dst.shape[1] // size
    dst[blk // nper, _blk(blk % nper, size)] = val


def _loop(lo, hi, body, unroll=1):
    def wrapped(i, carry):
        body(i)
        return carry

    jax.lax.fori_loop(lo, hi, wrapped, 0, unroll=unroll)


def _kernel(
    xa_h, kc_h, vc_h, wq_h, wo_h, xb_h, ckv_h, wbq_h, wuk_h, wuv_h, wbo_h, g_h,
    out_h, dxa_h, dk_h, dv_h, dwq_h, dwo_h, dxb_h, dckv_h, dwbq_h, dwuk_h, dwuv_h, dwbo_h,
    xa_v, xb_v, g_v, k_v, v_v, wq_v, wo_v, ckv_v, wbq_v, wu_v, wbo_v,
    out_v, dxa_v, dxb_v, dk_v, dv_v, dwq_v, dwo_v, dckv_v, dwbq_v, dwu_v, dwbo_v, z_v,
    colb_v, e_v, qd_v, rq_v, qb_v, sd_v, pd_v, pcd_v, acc_v, t_v, row_v, s_v, dp_v,
    qa_v, doa_v, oa_v, dqa_v,
    sem,
):
    def cp(src, dst, i):
        return pltpu.make_async_copy(src, dst, sem.at[i])

    def start_rows(src, dst, size, i):
        for j in range(0, dst.shape[0], size):
            cp(src.at[pl.ds(j, size)], dst.at[pl.ds(j, size)], i).start()

    def window(cache, h0, h1):
        return cache.at[0, pl.ds(h0, h1 - h0), pl.ds(W0, W), :]

    def start_window(cache, dst, h0, h1, i):
        for h in range(h0, h1):
            cp(cache.at[0, h, pl.ds(W0, W), :], dst.at[h], i).start()

    def wait_all(src, dst, i):
        cp(src, dst, i).wait()

    def start_zero(lo, hi, unrolled=False):
        for a, dst in enumerate((dk_h, dv_h)):
            l, u = max(lo - a * NZ, 0), min(hi - a * NZ, NZ)
            if l >= u:
                continue
            if unrolled:
                for i in range(l, u):
                    cp(z_v, dst.at[0, pl.ds(i // NZ_ROWS * NS, NS), pl.ds(i % NZ_ROWS * ZR, ZR), :],
                       W_SEM).start()
            else:
                def body(i, dst=dst):
                    cp(z_v, dst.at[0, _blk(i // NZ_ROWS, NS), _blk(i % NZ_ROWS, ZR), :], W_SEM).start()

                _loop(l, u, body)

    def start_window_grad(src, dst):
        nr = W // ZR

        def body(i):
            hs, r = _blk(i // nr, NS), i % nr
            cp(src.at[hs, _blk(r, ZR), :],
               dst.at[0, hs, pl.ds(pl.multiple_of(W0 + r * ZR, ZR), ZR), :], W_SEM).start()

        _loop(0, (H // NS) * nr, body)

    def start_streams(src, dst, size):
        def body(j):
            cp(src.at[:, _blk(j, size)], dst.at[:, _blk(j, size)], W_SEM).start()

        _loop(0, dst.shape[1] // size, body)

    cp(wbq_h.at[pl.ds(0, 128)], wbq_v.at[pl.ds(0, 128)], 0).start()
    cp(xa_h, xa_v, 0).start()
    cp(xb_h, xb_v, 0).start()
    cp(g_h, g_v, 0).start()
    start_rows(wbq_h.at[pl.ds(128, M - 128)], wbq_v.at[pl.ds(128, M - 128)], 128, 0)
    start_rows(wuk_h, wu_v.at[0], 128, 1)
    start_rows(wbo_h, wbo_v, HG, 2)
    start_rows(wuv_h, wu_v.at[1], 128, 3)

    z_v[...] = jnp.zeros(z_v.shape, bf16)

    def e_body(j):
        e_v[_blk(j, 512), :] = jnp.where(
            _iota((512, 128), 1) == (_iota((512, 128), 0) + j * 512) // H, 1.0, 0.0).astype(bf16)

    _loop(0, HD // 512, e_body)

    wait_all(wbq_h, wbq_v, 0)
    wait_all(xa_h, xa_v, 0)
    wait_all(xb_h, xb_v, 0)
    wait_all(g_h, g_v, 0)
    start_rows(ckv_h.at[0], ckv_v, 1024, 0)
    colb_v[0] = jnp.broadcast_to(xa_v[0].astype(f32), (128, M)).T
    colb_v[1] = jnp.broadcast_to(xb_v[0].astype(f32), (128, M)).T

    def qb_body(i, acc):
        r = _blk(i, MB)
        return acc + jnp.sum(wbq_v[r].astype(f32) * colb_v[1, r, :][:, None, :], axis=0)

    qb_v[0] = jax.lax.fori_loop(0, M // MB, qb_body, jnp.zeros((H, D), f32))

    def absorb(a):
        vec = qb_v[a].astype(bf16)
        own_head = _iota((H, HD), 1) % H == _iota((H, HD), 0)

        def body(j):
            w2 = wu_v[a, pl.ds(j * 128, 128)].reshape(HD, D)
            r = jnp.where(own_head, _dot_nt(vec, w2), 0.0).astype(bf16)
            qd_v[pl.ds(a * H, H), _blk(j, 128)] = _dot(r, e_v[...])

        _loop(0, C // 128, body)

    def project_back(row, load_w, dst):
        def body(j):
            dst[_blk(j, HG), :] = _dot_nt(row, load_w(j)).reshape(HG, D)

        _loop(0, H // HG, body)

    def project_out(src, load_w):
        def body(j, acc):
            return acc + _dot(src[_blk(j, HG), :].reshape(1, KC).astype(bf16), load_w(j))

        return jax.lax.fori_loop(0, H // HG, body, jnp.zeros((1, M), f32))

    def load_wbo(j):
        return wbo_v[pl.ds(j * HG, HG)].reshape(KC, M)

    def load_wo(j):
        return wo_v[_blk(j, KC), :]

    wait_all(wuk_h, wu_v.at[0], 1)
    start_rows(wq_h, wq_v, 128, 1)
    absorb(0)

    wait_all(wbo_h, wbo_v, 2)
    start_rows(wo_h, wo_v, 1024, 2)
    project_back(g_v[0][:, M:], load_wbo, qb_v.at[1])

    wait_all(wuv_h, wu_v.at[1], 3)
    start_window(kc_h, k_v, 0, H, 3)
    absorb(1)

    wait_all(ckv_h.at[0], ckv_v, 0)
    start_window(vc_h, v_v, 0, H - V_LATE, 0)
    qd = qd_v[...].astype(bf16)
    rq_v[...] = jnp.concatenate([qd[H:], qd[:H]], axis=0)

    def sd_body(j):
        sd_v[:, _blk(j, KC)] = _dot_nt(qd, ckv_v[_blk(j, KC), :])

    _loop(0, SK // KC, sd_body)

    def smx_body(j):
        lo = _blk(j, 16)
        hi = pl.ds(pl.multiple_of(H + j * 16, 16), 16)
        p = _softmax_rows(sd_v[lo, :] * SCALE)
        pd_v[lo, :] = p.astype(bf16)
        pd_v[hi, :] = _softmax_bwd_rows(p, sd_v[hi, :]).astype(bf16)

    _loop(0, H // 16, smx_body)

    def pc_body(j, acc):
        return acc + _dot(pd_v[:, _blk(j, KC)], ckv_v[_blk(j, KC), :])

    pcd_v[...] = jax.lax.fori_loop(0, SK // KC, pc_body, jnp.zeros((2 * H, C), f32))

    def unabsorb_body(it):
        a = it // 4
        j = it % 4
        blk = pcd_v[_blk(1 - a, H), _blk(j, 128)]
        vec = qb_v[a]
        acc = acc_v[a]
        per = C // NS
        for cc in range(128):
            col = jnp.broadcast_to(blk[:, cc:cc + 1], (H, D))
            dwu_v[a, j * (128 // per) + cc // per, cc % per] = (col * vec).astype(bf16)
            acc = acc + col * wu_v[a, j * 128 + cc].astype(f32)
        acc_v[a] = acc

    acc_v[...] = jnp.zeros(acc_v.shape, f32)
    _loop(0, 8, unabsorb_body)

    wait_all(wq_h, wq_v, 1)
    start_window(vc_h, v_v, H - V_LATE, H, 1)

    def qa_body(j):
        qa_v[_blk(j, HG), :] = _dot(xa_v[0], wq_v[:, _blk(j, KC)]).reshape(HG, D)

    _loop(0, H // HG, qa_body)

    dqb = acc_v[0]

    def dwbq_body(i):
        r = _blk(i, MB)
        _put_rows(dwbq_v, i, MB, (colb_v[1, r, :][:, None, :] * dqb[None]).astype(bf16))
        t_v[r, :] = jnp.sum(wbq_v[r].astype(f32) * dqb[None], axis=1)

    _loop(0, M // MB, dwbq_body)
    dxb_v[0] = jax.lax.dot_general(
        jnp.ones((8, D), f32), t_v[...], NT, preferred_element_type=f32,
        precision=jax.lax.Precision.HIGHEST)[0:1].astype(bf16)

    wait_all(wo_h, wo_v, 2)
    project_back(g_v[0][:, :M], load_wo, doa_v)

    def dckv_body(i):
        _put_rows(dckv_v, i, 512, _dot_tn(pd_v[:, _blk(i, 512)], rq_v[...]).astype(bf16))

    _loop(0, SK // 512, dckv_body)

    wait_all(window(kc_h, 0, H), k_v, 3)

    def s_body(h):
        s_v[pl.ds(h, 1), :] = _dot_nt(qa_v[pl.ds(h, 1), :].astype(bf16), k_v[h])

    _loop(0, H, s_body, unroll=2)
    s_v[...] = _softmax_rows(s_v[...] * SCALE)

    wait_all(window(vc_h, 0, H - V_LATE), v_v.at[pl.ds(0, H - V_LATE)], 0)
    start_zero(0, Z_TOPUP[0], unrolled=True)
    wait_all(window(vc_h, H - V_LATE, H), v_v.at[pl.ds(H - V_LATE, V_LATE)], 1)

    def dpo_body(h):
        vh = v_v[h]
        dp_v[pl.ds(h, 1), :] = _dot_nt(doa_v[pl.ds(h, 1), :].astype(bf16), vh)
        oa_v[pl.ds(h, 1), :] = _dot(s_v[pl.ds(h, 1), :].astype(bf16), vh)

    _loop(0, H, dpo_body, unroll=2)
    dp_v[...] = _softmax_bwd_rows(s_v[...], dp_v[...])
    start_zero(Z_TOPUP[0], Z_TOPUP[1])

    def dq_body(h):
        dqa_v[pl.ds(h, 1), :] = _dot(dp_v[pl.ds(h, 1), :].astype(bf16), k_v[h])

    _loop(0, H, dq_body, unroll=2)
    start_zero(Z_TOPUP[1], Z_TOPUP[2])

    def dkv_body(i):
        r = _blk(i, RB)
        p_t = s_v[:, r].T
        ds_t = dp_v[:, r].T.astype(bf16)
        head = _iota((H, D), 0)
        qa = qa_v[...]
        for h in range(H):
            dv_v[h, r, :] = (p_t[:, h:h + 1] * doa_v[h:h + 1, :]).astype(bf16)
            dk_v[h, r, :] = _dot(ds_t, jnp.where(head == h, qa, 0.0).astype(bf16)).astype(bf16)

    _loop(0, W // RB // 2, dkv_body)
    start_zero(Z_TOPUP[2], Z_TOPUP[3])
    _loop(W // RB // 2, W // RB, dkv_body)
    start_zero(Z_TOPUP[3], Z_TOPUP[4])

    row_v[...] = dqa_v[...].reshape(1, HD)
    out_a = project_out(oa_v, load_wo)
    out_b = project_out(acc_v.at[1], load_wbo)
    out_v[0] = jnp.concatenate([out_a, out_b], axis=1).astype(bf16)

    def dxa_body(j, acc):
        return acc + _dot_nt(row_v[:, _blk(j, KC)].astype(bf16), wq_v[:, _blk(j, KC)])

    dxa_v[0] = jax.lax.fori_loop(0, HD // KC, dxa_body, jnp.zeros((1, M), f32)).astype(bf16)

    def dwq_body(i):
        xcol = colb_v[0, _blk(i, MB), :]
        _put_rows(dwq_v, i, MB, (jnp.concatenate([xcol] * H, axis=1) * row_v[...]).astype(bf16))

    _loop(0, M // MB, dwq_body)

    def outer(col_ref, grow, dst):
        growf = grow.astype(f32)

        def body(h):
            cb = jnp.broadcast_to(col_ref[pl.ds(h, 1), :], (D, D)).T
            _put_rows(dst, h, D, (jnp.concatenate([cb] * (M // 128), axis=1) * growf).astype(bf16))

        _loop(0, H, body)

    start_zero(Z_TOPUP[4], Z_TOPUP[5])
    outer(oa_v, g_v[0][:, :M], dwo_v)
    start_zero(Z_TOPUP[5], Z_TOPUP[6])
    outer(acc_v.at[1], g_v[0][:, M:], dwbo_v)

    start_zero(Z_TOPUP[6], 2 * NZ)
    start_window_grad(dk_v, dk_h)
    start_window_grad(dv_v, dv_h)
    cp(dxa_v, dxa_h, W_SEM).start()
    cp(dxb_v, dxb_h, W_SEM).start()
    cp(out_v, out_h, W_SEM).start()

    def dwq_issue(i):
        r, c = _blk(i // 4, 8), _blk(i % 4, 1024)
        cp(dwq_v.at[:, r, c], dwq_h.at[:, r, c], W_SEM).start()

    _loop(0, dwq_h.shape[1] // 8 * 4, dwq_issue)
    start_streams(dwo_v, dwo_h, 16)
    start_streams(dwu_v.at[0], dwuk_h, 2)
    start_streams(dwu_v.at[1], dwuv_h, 2)
    start_streams(dwbq_v, dwbq_h, 2)
    start_streams(dwbo_v, dwbo_h, 16)
    start_streams(dckv_v, dckv_h, 16)

    for src, dst in ((dk_h, dk_h), (dv_h, dv_h), (dxa_v, dxa_h), (dxb_v, dxb_h), (out_v, out_h),
                     (dwq_v, dwq_h), (dwo_v, dwo_h), (dwu_v.at[0], dwuk_h), (dwu_v.at[1], dwuv_h),
                     (dwbq_v, dwbq_h), (dwbo_v, dwbo_h), (dckv_v, dckv_h)):
        wait_all(src, dst, W_SEM)


def _forward_backward(A_x, A_k_cache, A_v_cache, A_wq, A_wo, B_x, B_c_kv, B_w_q, B_w_uk, B_w_uv,
                      B_w_o, grad_out):
    sds = jax.ShapeDtypeStruct
    sh_dwq = (NS, M // NS, HD)
    sh_dwo = (NS, HD // NS, M)
    sh_dckv = (NS, SK // NS, C)
    sh_dwbq = (NS, M // NS, H, D)
    sh_dwu = (NS, C // NS, H, D)
    out_shape = (
        sds((1, 1, 2 * M), bf16), sds((1, 1, M), bf16),
        sds((1, H, SK, D), bf16), sds((1, H, SK, D), bf16),
        sds(sh_dwq, bf16), sds(sh_dwo, bf16),
        sds((1, 1, M), bf16), sds(sh_dckv, bf16),
        sds(sh_dwbq, bf16), sds(sh_dwu, bf16), sds(sh_dwu, bf16), sds(sh_dwo, bf16),
    )
    vm = pltpu.VMEM
    scratch = [
        vm((1, 1, M), bf16), vm((1, 1, M), bf16), vm((1, 1, 2 * M), bf16),
        vm((H, W, D), bf16), vm((H, W, D), bf16),
        vm((M, HD), bf16), vm((HD, M), bf16), vm((SK, C), bf16),
        vm((M, H, D), bf16), vm((2, C, H, D), bf16), vm((H, D, M), bf16),
        vm((1, 1, 2 * M), bf16), vm((1, 1, M), bf16), vm((1, 1, M), bf16),
        vm((H, W, D), bf16), vm((H, W, D), bf16),
        vm(sh_dwq, bf16), vm(sh_dwo, bf16), vm(sh_dckv, bf16),
        vm(sh_dwbq, bf16), vm((2,) + sh_dwu, bf16), vm(sh_dwo, bf16),
        vm((NS, ZR, D), bf16),
        vm((2, M, 128), f32),
        vm((HD, 128), bf16),
        vm((2 * H, C), f32),
        vm((2 * H, C), bf16),
        vm((2, H, D), f32),
        vm((2 * H, SK), f32),
        vm((2 * H, SK), bf16),
        vm((2 * H, C), f32),
        vm((2, H, D), f32),
        vm((M, D), f32),
        vm((1, HD), f32),
        vm((H, W), f32),
        vm((H, W), f32),
        vm((H, D), f32), vm((H, D), f32), vm((H, D), f32), vm((H, D), f32),
        pltpu.SemaphoreType.DMA((4,)),
    ]
    any_spec = pl.BlockSpec(memory_space=pl.ANY)
    outs = pl.pallas_call(
        _kernel,
        out_shape=out_shape,
        in_specs=[any_spec] * 12,
        out_specs=[any_spec] * 12,
        scratch_shapes=scratch,
        compiler_params=pltpu.CompilerParams(vmem_limit_bytes=120 * 1024 * 1024),
    )(A_x, A_k_cache, A_v_cache, A_wq, A_wo, B_x, B_c_kv, B_w_q, B_w_uk, B_w_uv, B_w_o, grad_out)
    out, dxa, dk, dv, dwq, dwo, dxb, dckv, dwbq, dwuk, dwuv, dwbo = outs
    return (out, dxa, dk, dv, dwq.reshape(M, HD), dwo.reshape(HD, M), dxb,
            dckv.reshape(1, SK, C), dwbq.reshape(M, H, D), dwuk.reshape(C, H, D),
            dwuv.reshape(C, H, D), dwbo.reshape(H, D, M))


@jax.jit
def pallas_concat_heads__sliding_block_cached__compressed_kv_cla__decode_kernel(
    A_x, A_k_cache, A_v_cache, A_wq, A_wo, B_x, B_c_kv, B_w_q, B_w_uk, B_w_uv, B_w_o, grad_out,
):
    return _forward_backward(A_x, A_k_cache, A_v_cache, A_wq, A_wo, B_x, B_c_kv, B_w_q, B_w_uk,
                             B_w_uv, B_w_o, grad_out)
```

```python
import jax
import jax.numpy as jnp
import jax.experimental.pallas as pl
import jax.experimental.pallas.tpu as pltpu

bf16 = jnp.bfloat16
f32 = jnp.float32

H = 32
D = 128
M = 640
HD = H * D
SK = 4096
W = 1024
W0 = SK - W
C = 512
SCALE = D ** -0.5

MB = 16
HG = 8
KC = HG * D
RB = 128
NS = 8
NS5 = 5
NS4 = 4
ZR = 64
V_LATE = 2
NZ_ROWS = W0 // ZR
NZ = (H // NS) * NZ_ROWS
Z_TOPUP = (72, 108, 130, 165, 200, 240, 280)
W_SEM = 2

NT = (((1,), (1,)), ((), ()))
TN = (((0,), (0,)), ((), ()))


def _dot(a, b):
    return jnp.dot(a, b, preferred_element_type=f32)


def _dot_nt(a, b):
    return jax.lax.dot_general(a, b, NT, preferred_element_type=f32)


def _dot_tn(a, b):
    return jax.lax.dot_general(a, b, TN, preferred_element_type=f32)


def _iota(shape, dim):
    return jax.lax.broadcasted_iota(jnp.int32, shape, dim)


def _softmax_rows(s):
    e = jnp.exp(s - jnp.max(s, axis=1, keepdims=True))
    return e * (1.0 / jnp.sum(e, axis=1, keepdims=True))


def _softmax_bwd_rows(p, dp):
    return p * (dp - jnp.sum(p * dp, axis=1, keepdims=True)) * SCALE


def _blk(i, size):
    return pl.ds(pl.multiple_of(i * size, size), size)


def _put_rows(dst, blk, size, val):
    nper = dst.shape[1] // size
    dst[blk // nper, _blk(blk % nper, size)] = val


def _loop(lo, hi, body, unroll=1):
    def wrapped(i, carry):
        body(i)
        return carry

    jax.lax.fori_loop(lo, hi, wrapped, 0, unroll=unroll)


def _kernel(
    xa_h, kc_h, vc_h, wq_h, wo_h, xb_h, ckv_h, wbq_h, wuk_h, wuv_h, wbo_h, g_h,
    out_h, dxa_h, dk_h, dv_h, dwq_h, dwo_h, dxb_h, dckv_h, dwbq_h, dwuk_h, dwuv_h, dwbo_h,
    xa_v, xb_v, g_v, k_v, v_v, wq_v, wo_v, ckv_v, wbq_v, wu_v, wbo_v,
    out_v, dxa_v, dxb_v, dk_v, dv_v, dwq_v, dwo_v, dckv_v, dwbq_v, dwu_v, dwbo_v, z_v,
    colb_v, e_v, qd_v, rq_v, qb_v, sd_v, pd_v, pcd_v, acc_v, t_v, row_v, s_v, dp_v,
    qa_v, doa_v, oa_v, dqa_v,
    sem,
):
    def cp(src, dst, i):
        return pltpu.make_async_copy(src, dst, sem.at[i])

    def start_rows(src, dst, size, i):
        for j in range(0, dst.shape[0], size):
            cp(src.at[pl.ds(j, size)], dst.at[pl.ds(j, size)], i).start()

    def window(cache, h0, h1):
        return cache.at[0, pl.ds(h0, h1 - h0), pl.ds(W0, W), :]

    def start_window(cache, dst, h0, h1, i):
        for h in range(h0, h1):
            cp(cache.at[0, h, pl.ds(W0, W), :], dst.at[h], i).start()

    def wait_all(src, dst, i):
        cp(src, dst, i).wait()

    def start_zero(lo, hi, unrolled=False):
        for a, dst in enumerate((dk_h, dv_h)):
            l, u = max(lo - a * NZ, 0), min(hi - a * NZ, NZ)
            if l >= u:
                continue
            if unrolled:
                for i in range(l, u):
                    cp(z_v, dst.at[0, pl.ds(i // NZ_ROWS * NS, NS), pl.ds(i % NZ_ROWS * ZR, ZR), :],
                       W_SEM).start()
            else:
                def body(i, dst=dst):
                    cp(z_v, dst.at[0, _blk(i // NZ_ROWS, NS), _blk(i % NZ_ROWS, ZR), :], W_SEM).start()

                _loop(l, u, body)

    def start_window_grad(src, dst):
        nr = W // ZR

        def body(i):
            hs, r = _blk(i // nr, NS), i % nr
            cp(src.at[hs, _blk(r, ZR), :],
               dst.at[0, hs, pl.ds(pl.multiple_of(W0 + r * ZR, ZR), ZR), :], W_SEM).start()

        _loop(0, (H // NS) * nr, body)

    def start_streams(*arrays):
        def body(j):
            for src, dst, size in arrays:
                cp(src.at[:, _blk(j, size)], dst.at[:, _blk(j, size)], W_SEM).start()

        _loop(0, arrays[0][1].shape[1] // arrays[0][2], body)

    cp(wbq_h.at[pl.ds(0, 128)], wbq_v.at[pl.ds(0, 128)], 0).start()
    cp(xa_h, xa_v, 0).start()
    cp(xb_h, xb_v, 0).start()
    cp(g_h, g_v, 0).start()
    start_rows(wbq_h.at[pl.ds(128, M - 128)], wbq_v.at[pl.ds(128, M - 128)], 128, 0)
    start_rows(wuk_h, wu_v.at[0], 128, 1)
    start_rows(wbo_h, wbo_v, HG, 2)
    start_rows(wuv_h, wu_v.at[1], 128, 3)

    z_v[...] = jnp.zeros(z_v.shape, bf16)

    def e_body(j):
        e_v[_blk(j, 512), :] = jnp.where(
            _iota((512, 128), 1) == (_iota((512, 128), 0) + j * 512) // H, 1.0, 0.0).astype(bf16)

    _loop(0, HD // 512, e_body)

    wait_all(wbq_h, wbq_v, 0)
    wait_all(xa_h, xa_v, 0)
    wait_all(xb_h, xb_v, 0)
    wait_all(g_h, g_v, 0)
    start_rows(ckv_h.at[0], ckv_v, 1024, 0)
    colb_v[0] = jnp.broadcast_to(xa_v[0].astype(f32), (128, M)).T
    colb_v[1] = jnp.broadcast_to(xb_v[0].astype(f32), (128, M)).T

    def qb_body(i, acc):
        r = _blk(i, MB)
        return acc + jnp.sum(wbq_v[r].astype(f32) * colb_v[1, r, :][:, None, :], axis=0)

    qb_v[0] = jax.lax.fori_loop(0, M // MB, qb_body, jnp.zeros((H, D), f32))

    def absorb(a):
        vec = qb_v[a].astype(bf16)
        own_head = _iota((H, HD), 1) % H == _iota((H, HD), 0)

        def body(j):
            w2 = wu_v[a, pl.ds(j * 128, 128)].reshape(HD, D)
            r = jnp.where(own_head, _dot_nt(vec, w2), 0.0).astype(bf16)
            qd_v[pl.ds(a * H, H), _blk(j, 128)] = _dot(r, e_v[...])

        _loop(0, C // 128, body)

    def project_back(row, load_w, dst):
        def body(j):
            dst[_blk(j, HG), :] = _dot_nt(row, load_w(j)).reshape(HG, D)

        _loop(0, H // HG, body)

    def project_out(src, load_w):
        def body(j, acc):
            return acc + _dot(src[_blk(j, HG), :].reshape(1, KC).astype(bf16), load_w(j))

        return jax.lax.fori_loop(0, H // HG, body, jnp.zeros((1, M), f32))

    def load_wbo(j):
        return wbo_v[pl.ds(j * HG, HG)].reshape(KC, M)

    def load_wo(j):
        return wo_v[_blk(j, KC), :]

    wait_all(wuk_h, wu_v.at[0], 1)
    start_rows(wq_h, wq_v, 128, 1)
    absorb(0)

    wait_all(wbo_h, wbo_v, 2)
    start_rows(wo_h, wo_v, 1024, 2)
    project_back(g_v[0][:, M:], load_wbo, qb_v.at[1])

    wait_all(wuv_h, wu_v.at[1], 3)
    start_window(kc_h, k_v, 0, H, 3)
    absorb(1)

    wait_all(ckv_h.at[0], ckv_v, 0)
    start_window(vc_h, v_v, 0, H - V_LATE, 0)
    qd = qd_v[...].astype(bf16)
    rq_v[...] = jnp.concatenate([qd[H:], qd[:H]], axis=0)

    def sd_body(j):
        sd_v[:, _blk(j, KC)] = _dot_nt(qd, ckv_v[_blk(j, KC), :])

    _loop(0, SK // KC, sd_body)

    def smx_body(j):
        lo = _blk(j, 16)
        hi = pl.ds(pl.multiple_of(H + j * 16, 16), 16)
        p = _softmax_rows(sd_v[lo, :] * SCALE)
        pd_v[lo, :] = p.astype(bf16)
        pd_v[hi, :] = _softmax_bwd_rows(p, sd_v[hi, :]).astype(bf16)

    _loop(0, H // 16, smx_body)

    def pc_body(j, acc):
        return acc + _dot(pd_v[:, _blk(j, KC)], ckv_v[_blk(j, KC), :])

    pcd_v[...] = jax.lax.fori_loop(0, SK // KC, pc_body, jnp.zeros((2 * H, C), f32))

    def unabsorb_body(it):
        a = it // 4
        j = it % 4
        blk = pcd_v[_blk(1 - a, H), _blk(j, 128)]
        vec = qb_v[a]
        acc = acc_v[a]
        for cc in range(128):
            col = jnp.broadcast_to(blk[:, cc:cc + 1], (H, D))
            dwu_v[a, j, cc] = (col * vec).astype(bf16)
            acc = acc + col * wu_v[a, j * 128 + cc].astype(f32)
        acc_v[a] = acc

    acc_v[...] = jnp.zeros(acc_v.shape, f32)
    _loop(0, 8, unabsorb_body)

    wait_all(wq_h, wq_v, 1)
    start_window(vc_h, v_v, H - V_LATE, H, 1)

    def qa_body(j):
        qa_v[_blk(j, HG), :] = _dot(xa_v[0], wq_v[:, _blk(j, KC)]).reshape(HG, D)

    _loop(0, H // HG, qa_body)

    dqb = acc_v[0]

    def dwbq_body(i):
        r = _blk(i, MB)
        _put_rows(dwbq_v, i, MB, (colb_v[1, r, :][:, None, :] * dqb[None]).astype(bf16))
        t_v[r, :] = jnp.sum(wbq_v[r].astype(f32) * dqb[None], axis=1)

    _loop(0, M // MB, dwbq_body)
    dxb_v[0] = jax.lax.dot_general(
        jnp.ones((8, D), f32), t_v[...], NT, preferred_element_type=f32,
        precision=jax.lax.Precision.HIGHEST)[0:1].astype(bf16)

    wait_all(wo_h, wo_v, 2)
    project_back(g_v[0][:, :M], load_wo, doa_v)

    def dckv_body(i):
        _put_rows(dckv_v, i, 512, _dot_tn(pd_v[:, _blk(i, 512)], rq_v[...]).astype(bf16))

    _loop(0, SK // 512, dckv_body)

    wait_all(window(kc_h, 0, H), k_v, 3)

    def s_body(h):
        s_v[pl.ds(h, 1), :] = _dot_nt(qa_v[pl.ds(h, 1), :].astype(bf16), k_v[h])

    _loop(0, H, s_body, unroll=2)
    s_v[...] = _softmax_rows(s_v[...] * SCALE)

    wait_all(window(vc_h, 0, H - V_LATE), v_v.at[pl.ds(0, H - V_LATE)], 0)
    start_zero(0, Z_TOPUP[0], unrolled=True)
    wait_all(window(vc_h, H - V_LATE, H), v_v.at[pl.ds(H - V_LATE, V_LATE)], 1)

    def dpo_body(h):
        vh = v_v[h]
        dp_v[pl.ds(h, 1), :] = _dot_nt(doa_v[pl.ds(h, 1), :].astype(bf16), vh)
        oa_v[pl.ds(h, 1), :] = _dot(s_v[pl.ds(h, 1), :].astype(bf16), vh)

    _loop(0, H, dpo_body, unroll=2)
    dp_v[...] = _softmax_bwd_rows(s_v[...], dp_v[...])
    start_zero(Z_TOPUP[0], Z_TOPUP[1])

    def dq_body(h):
        dqa_v[pl.ds(h, 1), :] = _dot(dp_v[pl.ds(h, 1), :].astype(bf16), k_v[h])

    _loop(0, H, dq_body, unroll=2)
    start_zero(Z_TOPUP[1], Z_TOPUP[2])

    def dkv_body(i):
        r = _blk(i, RB)
        p_t = s_v[:, r].T
        ds_t = dp_v[:, r].T.astype(bf16)
        head = _iota((H, D), 0)
        qa = qa_v[...]
        for h in range(H):
            dv_v[h, r, :] = (p_t[:, h:h + 1] * doa_v[h:h + 1, :]).astype(bf16)
            dk_v[h, r, :] = _dot(ds_t, jnp.where(head == h, qa, 0.0).astype(bf16)).astype(bf16)

    _loop(0, W // RB // 2, dkv_body)
    start_zero(Z_TOPUP[2], Z_TOPUP[3])
    _loop(W // RB // 2, W // RB, dkv_body)
    start_zero(Z_TOPUP[3], Z_TOPUP[4])

    row_v[...] = dqa_v[...].reshape(1, HD)
    out_a = project_out(oa_v, load_wo)
    out_b = project_out(acc_v.at[1], load_wbo)
    out_v[0] = jnp.concatenate([out_a, out_b], axis=1).astype(bf16)

    def dxa_body(j, acc):
        return acc + _dot_nt(row_v[:, _blk(j, KC)].astype(bf16), wq_v[:, _blk(j, KC)])

    dxa_v[0] = jax.lax.fori_loop(0, HD // KC, dxa_body, jnp.zeros((1, M), f32)).astype(bf16)

    def dwq_body(i):
        xcol = colb_v[0, _blk(i, MB), :]
        _put_rows(dwq_v, i, MB, (jnp.concatenate([xcol] * H, axis=1) * row_v[...]).astype(bf16))

    _loop(0, M // MB, dwq_body)

    def outer(col_ref, grow, dst):
        growf = grow.astype(f32)

        def body(h):
            cb = jnp.broadcast_to(col_ref[pl.ds(h, 1), :], (D, D)).T
            _put_rows(dst, h, D, (jnp.concatenate([cb] * (M // 128), axis=1) * growf).astype(bf16))

        _loop(0, H, body)

    start_zero(Z_TOPUP[4], Z_TOPUP[5])
    outer(oa_v, g_v[0][:, :M], dwo_v)
    start_zero(Z_TOPUP[5], Z_TOPUP[6])
    outer(acc_v.at[1], g_v[0][:, M:], dwbo_v)

    start_zero(Z_TOPUP[6], 2 * NZ)
    start_window_grad(dk_v, dk_h)
    start_window_grad(dv_v, dv_h)
    cp(dxa_v, dxa_h, W_SEM).start()
    cp(dxb_v, dxb_h, W_SEM).start()
    cp(out_v, out_h, W_SEM).start()

    def dwq_issue(i):
        r, c = _blk(i // 4, 8), _blk(i % 4, 1024)
        cp(dwq_v.at[:, r, c], dwq_h.at[:, r, c], W_SEM).start()

    _loop(0, dwq_h.shape[1] // 8 * 4, dwq_issue)
    start_streams((dwbq_v, dwbq_h, 2))
    start_streams((dwo_v, dwo_h, 16), (dwbo_v, dwbo_h, 16))
    start_streams((dwu_v.at[0], dwuk_h, 2), (dwu_v.at[1], dwuv_h, 2), (dckv_v, dckv_h, 16))

    for src, dst in ((dk_h, dk_h), (dv_h, dv_h), (dxa_v, dxa_h), (dxb_v, dxb_h), (out_v, out_h),
                     (dwq_v, dwq_h), (dwo_v, dwo_h), (dwu_v.at[0], dwuk_h), (dwu_v.at[1], dwuv_h),
                     (dwbq_v, dwbq_h), (dwbo_v, dwbo_h), (dckv_v, dckv_h)):
        wait_all(src, dst, W_SEM)


def _forward_backward(A_x, A_k_cache, A_v_cache, A_wq, A_wo, B_x, B_c_kv, B_w_q, B_w_uk, B_w_uv,
                      B_w_o, grad_out):
    sds = jax.ShapeDtypeStruct
    sh_dwq = (NS5, M // NS5, HD)
    sh_dwo = (NS4, HD // NS4, M)
    sh_dckv = (NS4, SK // NS4, C)
    sh_dwbq = (NS5, M // NS5, H, D)
    sh_dwu = (NS4, C // NS4, H, D)
    out_shape = (
        sds((1, 1, 2 * M), bf16), sds((1, 1, M), bf16),
        sds((1, H, SK, D), bf16), sds((1, H, SK, D), bf16),
        sds(sh_dwq, bf16), sds(sh_dwo, bf16),
        sds((1, 1, M), bf16), sds(sh_dckv, bf16),
        sds(sh_dwbq, bf16), sds(sh_dwu, bf16), sds(sh_dwu, bf16), sds(sh_dwo, bf16),
    )
    vm = pltpu.VMEM
    scratch = [
        vm((1, 1, M), bf16), vm((1, 1, M), bf16), vm((1, 1, 2 * M), bf16),
        vm((H, W, D), bf16), vm((H, W, D), bf16),
        vm((M, HD), bf16), vm((HD, M), bf16), vm((SK, C), bf16),
        vm((M, H, D), bf16), vm((2, C, H, D), bf16), vm((H, D, M), bf16),
        vm((1, 1, 2 * M), bf16), vm((1, 1, M), bf16), vm((1, 1, M), bf16),
        vm((H, W, D), bf16), vm((H, W, D), bf16),
        vm(sh_dwq, bf16), vm(sh_dwo, bf16), vm(sh_dckv, bf16),
        vm(sh_dwbq, bf16), vm((2,) + sh_dwu, bf16), vm(sh_dwo, bf16),
        vm((NS, ZR, D), bf16),
        vm((2, M, 128), f32),
        vm((HD, 128), bf16),
        vm((2 * H, C), f32),
        vm((2 * H, C), bf16),
        vm((2, H, D), f32),
        vm((2 * H, SK), f32),
        vm((2 * H, SK), bf16),
        vm((2 * H, C), f32),
        vm((2, H, D), f32),
        vm((M, D), f32),
        vm((1, HD), f32),
        vm((H, W), f32),
        vm((H, W), f32),
        vm((H, D), f32), vm((H, D), f32), vm((H, D), f32), vm((H, D), f32),
        pltpu.SemaphoreType.DMA((4,)),
    ]
    any_spec = pl.BlockSpec(memory_space=pl.ANY)
    outs = pl.pallas_call(
        _kernel,
        out_shape=out_shape,
        in_specs=[any_spec] * 12,
        out_specs=[any_spec] * 12,
        scratch_shapes=scratch,
        compiler_params=pltpu.CompilerParams(vmem_limit_bytes=120 * 1024 * 1024),
    )(A_x, A_k_cache, A_v_cache, A_wq, A_wo, B_x, B_c_kv, B_w_q, B_w_uk, B_w_uv, B_w_o, grad_out)
    out, dxa, dk, dv, dwq, dwo, dxb, dckv, dwbq, dwuk, dwuv, dwbo = outs
    return (out, dxa, dk, dv, dwq.reshape(M, HD), dwo.reshape(HD, M), dxb,
            dckv.reshape(1, SK, C), dwbq.reshape(M, H, D), dwuk.reshape(C, H, D),
            dwuv.reshape(C, H, D), dwbo.reshape(H, D, M))


@jax.jit
def pallas_concat_heads__sliding_block_cached__compressed_kv_cla__decode_kernel(
    A_x, A_k_cache, A_v_cache, A_wq, A_wo, B_x, B_c_kv, B_w_q, B_w_uk, B_w_uv, B_w_o, grad_out,
):
    return _forward_backward(A_x, A_k_cache, A_v_cache, A_wq, A_wo, B_x, B_c_kv, B_w_q, B_w_uk,
                             B_w_uv, B_w_o, grad_out)
```

```python
import jax
import jax.numpy as jnp
import jax.experimental.pallas as pl
import jax.experimental.pallas.tpu as pltpu

bf16 = jnp.bfloat16
f32 = jnp.float32

H = 32
D = 128
M = 640
HD = H * D
SK = 4096
W = 1024
W0 = SK - W
C = 512
SCALE = D ** -0.5

MB = 16
HG = 8
KC = HG * D
RB = 128
NS5 = 5
NS4 = 4
HEAD_GROUPS = ((0, 7), (7, 7), (14, 6), (20, 6), (26, 6))
ZR = 64
NZ_ROWS = W0 // ZR
NZ = 2 * len(HEAD_GROUPS) * NZ_ROWS
Z_TOPUP = (72, 135, 163, 207, 250, 300, 350)
V_LATE = 2
W_SEM = 2

NT = (((1,), (1,)), ((), ()))
TN = (((0,), (0,)), ((), ()))


def _dot(a, b):
    return jnp.dot(a, b, preferred_element_type=f32)


def _dot_nt(a, b):
    return jax.lax.dot_general(a, b, NT, preferred_element_type=f32)


def _dot_tn(a, b):
    return jax.lax.dot_general(a, b, TN, preferred_element_type=f32)


def _iota(shape, dim):
    return jax.lax.broadcasted_iota(jnp.int32, shape, dim)


def _softmax_rows(s):
    e = jnp.exp(s - jnp.max(s, axis=1, keepdims=True))
    return e * (1.0 / jnp.sum(e, axis=1, keepdims=True))


def _softmax_bwd_rows(p, dp):
    return p * (dp - jnp.sum(p * dp, axis=1, keepdims=True)) * SCALE


def _blk(i, size):
    return pl.ds(pl.multiple_of(i * size, size), size)


def _put_rows(dst, blk, size, val):
    nper = dst.shape[1] // size
    dst[blk // nper, _blk(blk % nper, size)] = val


def _loop(lo, hi, body, unroll=1):
    def wrapped(i, carry):
        body(i)
        return carry

    jax.lax.fori_loop(lo, hi, wrapped, 0, unroll=unroll)


def _kernel(
    xa_h, kc_h, vc_h, wq_h, wo_h, xb_h, ckv_h, wbq_h, wuk_h, wuv_h, wbo_h, g_h,
    out_h, dxa_h, dk_h, dv_h, dwq_h, dwo_h, dxb_h, dckv_h, dwbq_h, dwuk_h, dwuv_h, dwbo_h,
    xa_v, xb_v, g_v, k_v, v_v, wq_v, wo_v, ckv_v, wbq_v, wu_v, wbo_v,
    out_v, dxa_v, dxb_v, dk_v, dv_v, dwq_v, dwo_v, dckv_v, dwbq_v, dwu_v, dwbo_v, z_v,
    colb_v, e_v, qd_v, rq_v, qb_v, sd_v, pd_v, pcd_v, acc_v, t_v, row_v, s_v, dp_v,
    qa_v, doa_v, oa_v, dqa_v,
    sem,
):
    def cp(src, dst, i):
        return pltpu.make_async_copy(src, dst, sem.at[i])

    def start_rows(src, dst, size, i):
        for j in range(0, dst.shape[0], size):
            cp(src.at[pl.ds(j, size)], dst.at[pl.ds(j, size)], i).start()

    def window(cache, h0, h1):
        return cache.at[0, pl.ds(h0, h1 - h0), pl.ds(W0, W), :]

    def start_window(cache, dst, h0, h1, i):
        for h in range(h0, h1):
            cp(cache.at[0, h, pl.ds(W0, W), :], dst.at[h], i).start()

    def wait_all(src, dst, i):
        cp(src, dst, i).wait()

    def start_zero(lo, hi, unrolled=False):
        parts = [(dst, h0, n) for dst in (dk_h, dv_h) for h0, n in HEAD_GROUPS]
        for k, (dst, h0, n) in enumerate(parts):
            first, last = max(lo - k * NZ_ROWS, 0), min(hi - k * NZ_ROWS, NZ_ROWS)
            if first >= last:
                continue
            src = z_v.at[pl.ds(0, n)]
            if unrolled:
                for i in range(first, last):
                    cp(src, dst.at[0, pl.ds(h0, n), pl.ds(i * ZR, ZR), :], W_SEM).start()
            else:
                def body(i, src=src, dst=dst, h0=h0, n=n):
                    cp(src, dst.at[0, pl.ds(h0, n), _blk(i, ZR), :], W_SEM).start()

                _loop(first, last, body)

    def start_window_grad(src, dst):
        for h0, n in HEAD_GROUPS:
            def body(r, h0=h0, n=n):
                cp(src.at[pl.ds(h0, n), _blk(r, ZR), :],
                   dst.at[0, pl.ds(h0, n), pl.ds(pl.multiple_of(W0 + r * ZR, ZR), ZR), :], W_SEM).start()

            _loop(0, W // ZR, body)

    def start_streams(*arrays):
        def body(j):
            for src, dst, size in arrays:
                cp(src.at[:, _blk(j, size)], dst.at[:, _blk(j, size)], W_SEM).start()

        _loop(0, arrays[0][1].shape[1] // arrays[0][2], body)

    cp(wbq_h.at[pl.ds(0, 128)], wbq_v.at[pl.ds(0, 128)], 0).start()
    cp(xa_h, xa_v, 0).start()
    cp(xb_h, xb_v, 0).start()
    cp(g_h, g_v, 0).start()
    start_rows(wbq_h.at[pl.ds(128, M - 128)], wbq_v.at[pl.ds(128, M - 128)], 128, 0)
    start_rows(wuk_h, wu_v.at[0], 128, 1)
    start_rows(wbo_h, wbo_v, HG, 2)
    start_rows(wuv_h, wu_v.at[1], 128, 3)

    z_v[...] = jnp.zeros(z_v.shape, bf16)

    def e_body(j):
        e_v[_blk(j, 512), :] = jnp.where(
            _iota((512, 128), 1) == (_iota((512, 128), 0) + j * 512) // H, 1.0, 0.0).astype(bf16)

    _loop(0, HD // 512, e_body)

    wait_all(wbq_h, wbq_v, 0)
    wait_all(xa_h, xa_v, 0)
    wait_all(xb_h, xb_v, 0)
    wait_all(g_h, g_v, 0)
    start_rows(ckv_h.at[0], ckv_v, 1024, 0)
    colb_v[0] = jnp.broadcast_to(xa_v[0].astype(f32), (128, M)).T
    colb_v[1] = jnp.broadcast_to(xb_v[0].astype(f32), (128, M)).T

    def qb_body(i, acc):
        r = _blk(i, MB)
        return acc + jnp.sum(wbq_v[r].astype(f32) * colb_v[1, r, :][:, None, :], axis=0)

    qb_v[0] = jax.lax.fori_loop(0, M // MB, qb_body, jnp.zeros((H, D), f32))

    def absorb(a):
        vec = qb_v[a].astype(bf16)
        own_head = _iota((H, HD), 1) % H == _iota((H, HD), 0)

        def body(j):
            w2 = wu_v[a, pl.ds(j * 128, 128)].reshape(HD, D)
            r = jnp.where(own_head, _dot_nt(vec, w2), 0.0).astype(bf16)
            qd_v[pl.ds(a * H, H), _blk(j, 128)] = _dot(r, e_v[...])

        _loop(0, C // 128, body)

    def project_back(row, load_w, dst):
        def body(j):
            dst[_blk(j, HG), :] = _dot_nt(row, load_w(j)).reshape(HG, D)

        _loop(0, H // HG, body)

    def project_out(src, load_w):
        def body(j, acc):
            return acc + _dot(src[_blk(j, HG), :].reshape(1, KC).astype(bf16), load_w(j))

        return jax.lax.fori_loop(0, H // HG, body, jnp.zeros((1, M), f32))

    def load_wbo(j):
        return wbo_v[pl.ds(j * HG, HG)].reshape(KC, M)

    def load_wo(j):
        return wo_v[_blk(j, KC), :]

    wait_all(wuk_h, wu_v.at[0], 1)
    start_rows(wq_h, wq_v, 128, 1)
    absorb(0)

    wait_all(wbo_h, wbo_v, 2)
    start_rows(wo_h, wo_v, 1024, 2)
    project_back(g_v[0][:, M:], load_wbo, qb_v.at[1])

    wait_all(wuv_h, wu_v.at[1], 3)
    start_window(kc_h, k_v, 0, H, 3)
    absorb(1)

    wait_all(ckv_h.at[0], ckv_v, 0)
    start_window(vc_h, v_v, 0, H - V_LATE, 0)
    qd = qd_v[...].astype(bf16)
    rq_v[...] = jnp.concatenate([qd[H:], qd[:H]], axis=0)

    def sd_body(j):
        sd_v[:, _blk(j, KC)] = _dot_nt(qd, ckv_v[_blk(j, KC), :])

    _loop(0, SK // KC, sd_body)

    def smx_body(j):
        lo = _blk(j, 16)
        hi = pl.ds(pl.multiple_of(H + j * 16, 16), 16)
        p = _softmax_rows(sd_v[lo, :] * SCALE)
        pd_v[lo, :] = p.astype(bf16)
        pd_v[hi, :] = _softmax_bwd_rows(p, sd_v[hi, :]).astype(bf16)

    _loop(0, H // 16, smx_body)

    def pc_body(j, acc):
        return acc + _dot(pd_v[:, _blk(j, KC)], ckv_v[_blk(j, KC), :])

    pcd_v[...] = jax.lax.fori_loop(0, SK // KC, pc_body, jnp.zeros((2 * H, C), f32))

    def unabsorb_body(it):
        a = it // 4
        j = it % 4
        blk = pcd_v[_blk(1 - a, H), _blk(j, 128)]
        vec = qb_v[a]
        acc = acc_v[a]
        for cc in range(128):
            col = jnp.broadcast_to(blk[:, cc:cc + 1], (H, D))
            dwu_v[a, j, cc] = (col * vec).astype(bf16)
            acc = acc + col * wu_v[a, j * 128 + cc].astype(f32)
        acc_v[a] = acc

    acc_v[...] = jnp.zeros(acc_v.shape, f32)
    _loop(0, 8, unabsorb_body)

    wait_all(wq_h, wq_v, 1)
    start_window(vc_h, v_v, H - V_LATE, H, 1)

    def qa_body(j):
        qa_v[_blk(j, HG), :] = _dot(xa_v[0], wq_v[:, _blk(j, KC)]).reshape(HG, D)

    _loop(0, H // HG, qa_body)

    dqb = acc_v[0]

    def dwbq_body(i):
        r = _blk(i, MB)
        _put_rows(dwbq_v, i, MB, (colb_v[1, r, :][:, None, :] * dqb[None]).astype(bf16))
        t_v[r, :] = jnp.sum(wbq_v[r].astype(f32) * dqb[None], axis=1)

    _loop(0, M // MB, dwbq_body)
    dxb_v[0] = jax.lax.dot_general(
        jnp.ones((8, D), f32), t_v[...], NT, preferred_element_type=f32,
        precision=jax.lax.Precision.HIGHEST)[0:1].astype(bf16)

    wait_all(wo_h, wo_v, 2)
    project_back(g_v[0][:, :M], load_wo, doa_v)

    def dckv_body(i):
        _put_rows(dckv_v, i, 512, _dot_tn(pd_v[:, _blk(i, 512)], rq_v[...]).astype(bf16))

    _loop(0, SK // 512, dckv_body)

    wait_all(window(kc_h, 0, H), k_v, 3)

    def s_body(h):
        s_v[pl.ds(h, 1), :] = _dot_nt(qa_v[pl.ds(h, 1), :].astype(bf16), k_v[h])

    _loop(0, H, s_body, unroll=2)
    s_v[...] = _softmax_rows(s_v[...] * SCALE)

    wait_all(window(vc_h, 0, H - V_LATE), v_v.at[pl.ds(0, H - V_LATE)], 0)
    start_zero(0, Z_TOPUP[0], unrolled=True)
    wait_all(window(vc_h, H - V_LATE, H), v_v.at[pl.ds(H - V_LATE, V_LATE)], 1)

    def dpo_body(h):
        vh = v_v[h]
        dp_v[pl.ds(h, 1), :] = _dot_nt(doa_v[pl.ds(h, 1), :].astype(bf16), vh)
        oa_v[pl.ds(h, 1), :] = _dot(s_v[pl.ds(h, 1), :].astype(bf16), vh)

    _loop(0, H, dpo_body, unroll=2)
    dp_v[...] = _softmax_bwd_rows(s_v[...], dp_v[...])
    start_zero(Z_TOPUP[0], Z_TOPUP[1])

    def dq_body(h):
        dqa_v[pl.ds(h, 1), :] = _dot(dp_v[pl.ds(h, 1), :].astype(bf16), k_v[h])

    _loop(0, H, dq_body, unroll=2)
    start_zero(Z_TOPUP[1], Z_TOPUP[2])

    def dkv_body(i):
        r = _blk(i, RB)
        p_t = s_v[:, r].T
        ds_t = dp_v[:, r].T.astype(bf16)
        head = _iota((H, D), 0)
        qa = qa_v[...]
        for h in range(H):
            dv_v[h, r, :] = (p_t[:, h:h + 1] * doa_v[h:h + 1, :]).astype(bf16)
            dk_v[h, r, :] = _dot(ds_t, jnp.where(head == h, qa, 0.0).astype(bf16)).astype(bf16)

    _loop(0, W // RB // 2, dkv_body)
    start_zero(Z_TOPUP[2], Z_TOPUP[3])
    _loop(W // RB // 2, W // RB, dkv_body)
    start_zero(Z_TOPUP[3], Z_TOPUP[4])

    row_v[...] = dqa_v[...].reshape(1, HD)
    out_a = project_out(oa_v, load_wo)
    out_b = project_out(acc_v.at[1], load_wbo)
    out_v[0] = jnp.concatenate([out_a, out_b], axis=1).astype(bf16)

    def dxa_body(j, acc):
        return acc + _dot_nt(row_v[:, _blk(j, KC)].astype(bf16), wq_v[:, _blk(j, KC)])

    dxa_v[0] = jax.lax.fori_loop(0, HD // KC, dxa_body, jnp.zeros((1, M), f32)).astype(bf16)

    def dwq_body(i):
        xcol = colb_v[0, _blk(i, MB), :]
        _put_rows(dwq_v, i, MB, (jnp.concatenate([xcol] * H, axis=1) * row_v[...]).astype(bf16))

    _loop(0, M // MB, dwq_body)

    def outer(col_ref, grow, dst):
        growf = grow.astype(f32)

        def body(h):
            cb = jnp.broadcast_to(col_ref[pl.ds(h, 1), :], (D, D)).T
            _put_rows(dst, h, D, (jnp.concatenate([cb] * (M // 128), axis=1) * growf).astype(bf16))

        _loop(0, H, body)

    start_zero(Z_TOPUP[4], Z_TOPUP[5])
    outer(oa_v, g_v[0][:, :M], dwo_v)
    start_zero(Z_TOPUP[5], Z_TOPUP[6])
    outer(acc_v.at[1], g_v[0][:, M:], dwbo_v)

    start_zero(Z_TOPUP[6], NZ)
    start_window_grad(dk_v, dk_h)
    start_window_grad(dv_v, dv_h)
    cp(dxa_v, dxa_h, W_SEM).start()
    cp(dxb_v, dxb_h, W_SEM).start()
    cp(out_v, out_h, W_SEM).start()

    def dwq_issue(i):
        r, c = _blk(i // 4, 8), _blk(i % 4, 1024)
        cp(dwq_v.at[:, r, c], dwq_h.at[:, r, c], W_SEM).start()

    _loop(0, dwq_h.shape[1] // 8 * 4, dwq_issue)
    start_streams((dwbq_v, dwbq_h, 2))
    start_streams((dwo_v, dwo_h, 16), (dwbo_v, dwbo_h, 16))
    start_streams((dwu_v.at[0], dwuk_h, 2), (dwu_v.at[1], dwuv_h, 2), (dckv_v, dckv_h, 16))

    for src, dst in ((dk_h, dk_h), (dv_h, dv_h), (dxa_v, dxa_h), (dxb_v, dxb_h), (out_v, out_h),
                     (dwq_v, dwq_h), (dwo_v, dwo_h), (dwu_v.at[0], dwuk_h), (dwu_v.at[1], dwuv_h),
                     (dwbq_v, dwbq_h), (dwbo_v, dwbo_h), (dckv_v, dckv_h)):
        wait_all(src, dst, W_SEM)


def _forward_backward(A_x, A_k_cache, A_v_cache, A_wq, A_wo, B_x, B_c_kv, B_w_q, B_w_uk, B_w_uv,
                      B_w_o, grad_out):
    sds = jax.ShapeDtypeStruct
    sh_dwq = (NS5, M // NS5, HD)
    sh_dwo = (NS4, HD // NS4, M)
    sh_dckv = (NS4, SK // NS4, C)
    sh_dwbq = (NS5, M // NS5, H, D)
    sh_dwu = (NS4, C // NS4, H, D)
    out_shape = (
        sds((1, 1, 2 * M), bf16), sds((1, 1, M), bf16),
        sds((1, H, SK, D), bf16), sds((1, H, SK, D), bf16),
        sds(sh_dwq, bf16), sds(sh_dwo, bf16),
        sds((1, 1, M), bf16), sds(sh_dckv, bf16),
        sds(sh_dwbq, bf16), sds(sh_dwu, bf16), sds(sh_dwu, bf16), sds(sh_dwo, bf16),
    )
    vm = pltpu.VMEM
    scratch = [
        vm((1, 1, M), bf16), vm((1, 1, M), bf16), vm((1, 1, 2 * M), bf16),
        vm((H, W, D), bf16), vm((H, W, D), bf16),
        vm((M, HD), bf16), vm((HD, M), bf16), vm((SK, C), bf16),
        vm((M, H, D), bf16), vm((2, C, H, D), bf16), vm((H, D, M), bf16),
        vm((1, 1, 2 * M), bf16), vm((1, 1, M), bf16), vm((1, 1, M), bf16),
        vm((H, W, D), bf16), vm((H, W, D), bf16),
        vm(sh_dwq, bf16), vm(sh_dwo, bf16), vm(sh_dckv, bf16),
        vm(sh_dwbq, bf16), vm((2,) + sh_dwu, bf16), vm(sh_dwo, bf16),
        vm((max(n for _, n in HEAD_GROUPS), ZR, D), bf16),
        vm((2, M, 128), f32),
        vm((HD, 128), bf16),
        vm((2 * H, C), f32),
        vm((2 * H, C), bf16),
        vm((2, H, D), f32),
        vm((2 * H, SK), f32),
        vm((2 * H, SK), bf16),
        vm((2 * H, C), f32),
        vm((2, H, D), f32),
        vm((M, D), f32),
        vm((1, HD), f32),
        vm((H, W), f32),
        vm((H, W), f32),
        vm((H, D), f32), vm((H, D), f32), vm((H, D), f32), vm((H, D), f32),
        pltpu.SemaphoreType.DMA((4,)),
    ]
    any_spec = pl.BlockSpec(memory_space=pl.ANY)
    outs = pl.pallas_call(
        _kernel,
        out_shape=out_shape,
        in_specs=[any_spec] * 12,
        out_specs=[any_spec] * 12,
        scratch_shapes=scratch,
        compiler_params=pltpu.CompilerParams(vmem_limit_bytes=120 * 1024 * 1024),
    )(A_x, A_k_cache, A_v_cache, A_wq, A_wo, B_x, B_c_kv, B_w_q, B_w_uk, B_w_uv, B_w_o, grad_out)
    out, dxa, dk, dv, dwq, dwo, dxb, dckv, dwbq, dwuk, dwuv, dwbo = outs
    return (out, dxa, dk, dv, dwq.reshape(M, HD), dwo.reshape(HD, M), dxb,
            dckv.reshape(1, SK, C), dwbq.reshape(M, H, D), dwuk.reshape(C, H, D),
            dwuv.reshape(C, H, D), dwbo.reshape(H, D, M))


@jax.jit
def pallas_concat_heads__sliding_block_cached__compressed_kv_cla__decode_kernel(
    A_x, A_k_cache, A_v_cache, A_wq, A_wo, B_x, B_c_kv, B_w_q, B_w_uk, B_w_uv, B_w_o, grad_out,
):
    return _forward_backward(A_x, A_k_cache, A_v_cache, A_wq, A_wo, B_x, B_c_kv, B_w_q, B_w_uk,
                             B_w_uv, B_w_o, grad_out)
```
